```python
import jax
import jax.numpy as jnp

def _softmax(x, axis=-1):
    return jax.nn.softmax(x, axis=axis)

def _gelu(x):
    return jax.nn.gelu(x, approximate=True)

def _silu(x):
    return jax.nn.silu(x)

def _sigmoid(x):
    return jax.nn.sigmoid(x)

def _layernorm(x, axis=-1, eps=1e-05):
    m = jnp.mean(x, axis=axis, keepdims=True)
    v = jnp.var(x, axis=axis, keepdims=True)
    return (x - m) / jnp.sqrt(v + eps)

def _scatter_add(tgt, idx, src, axis=0):
    return tgt.at[idx].add(src)

def _segment_sum(src, seg, n):
    return jax.ops.segment_sum(src, seg, n)

class _Rng:

    def __init__(self, key):
        self._k = key

    def _next(self):
        self._k, sub = jax.random.split(self._k)
        return sub

    def normal(self, shape):
        return jax.random.normal(self._next(), shape, dtype=jnp.bfloat16)

    def randint(self, lo, hi, shape):
        return jax.random.randint(self._next(), shape, lo, hi, dtype=jnp.int32)

    def uniform(self, shape, lo=0.0, hi=1.0):
        return jax.random.uniform(self._next(), shape, jnp.bfloat16, lo, hi)

    def permutation(self, n):
        return jax.random.permutation(self._next(), n)
kernel_name = 'adaLN_cond__grouped_kv_mqa__mixer_token_mlp__prompt'

def _fwd_setup_inputs():
    _rng = _Rng(jax.random.key(int.from_bytes(__import__("os").urandom(4), "little")))
    _w = lambda a: (lambda t: t.astype(jnp.bfloat16) if jnp.issubdtype(t.dtype, jnp.floating) else t)(jnp.asarray(a))

    def _A_setup():
        B, S, D, H = (1, 2048, 512, 32)
        Dh = D // H
        return {'x': _w((lambda *s: _rng.normal(s) * 0.05)(B, S, D)), 'wq': _w((lambda *s: _rng.normal(s) * 0.05)(D, H * Dh)), 'wk': _w((lambda *s: _rng.normal(s) * 0.05)(D, Dh)), 'wv': _w((lambda *s: _rng.normal(s) * 0.05)(D, Dh)), 'wo': _w((lambda *s: _rng.normal(s) * 0.05)(H * Dh, D))}
    _A_in = _A_setup()

    def _B_setup():
        B, S, D, F = (1, 2048, 512, 1376)
        return {'x': _w((lambda *s: _rng.normal(s) * 0.05)(B, S, D)), 'w1': _w((lambda *s: _rng.normal(s) * 0.05)(S, F) * S ** (-0.5)), 'b1': _w((lambda *s: _rng.normal(s) * 0.05)(F) * 0.02), 'w2': _w((lambda *s: _rng.normal(s) * 0.05)(F, S) * F ** (-0.5)), 'b2': _w((lambda *s: _rng.normal(s) * 0.05)(S) * 0.02)}
    _B_in = _B_setup()
    return {'A_x': _A_in['x'], 'A_wq': _A_in['wq'], 'A_wk': _A_in['wk'], 'A_wv': _A_in['wv'], 'A_wo': _A_in['wo'], 'B_x': _B_in['x'], 'B_w1': _B_in['w1'], 'B_b1': _B_in['b1'], 'B_w2': _B_in['w2'], 'B_b2': _B_in['b2'], 'c': _w((lambda *s: _rng.normal(s) * 0.05)(1, 512)), 'w_mod': _w((lambda *s: _rng.normal(s) * 0.05)(512, 6 * 512) * 512 ** (-0.5))}

def _fwd_reference(A_x, A_wq, A_wk, A_wv, A_wo, B_x, B_w1, B_b1, B_w2, B_b2, c, w_mod):

    def _A_ref(x, wq, wk, wv, wo):
        B, S, D = x.shape
        H = 32
        Dh = D // H
        q = (lambda x, *d: x.transpose(*d))((x @ wq).reshape(B, S, H, Dh), 0, 2, 1, 3)
        k = x @ wk
        v = x @ wv
        scores = jnp.einsum('bhqd,bkd->bhqk', q, k) * Dh ** (-0.5)
        p = _softmax(scores, axis=-1)
        o = jnp.einsum('bhqk,bkd->bhqd', p, v)
        return (lambda x, *d: x.transpose(*d))(o, 0, 2, 1, 3).reshape(B, S, H * Dh) @ wo

    def _B_ref(x, w1, b1, w2, b2):
        B, S, D = x.shape
        h = _layernorm(x, axis=-1)
        u = jnp.einsum('bsd,sf->bdf', h, w1) + b1
        u = _gelu(u)
        y = jnp.einsum('bdf,fs->bds', u, w2) + b2
        return (lambda x, *d: x.transpose(*d))(y, 0, 2, 1)
    x = A_x
    mod = (_silu(c) @ w_mod).reshape(c.shape[0], 6, 1, -1)
    sa, ca, ga, sb, cb, gb = (mod[:, 0].copy(), mod[:, 1].copy(), mod[:, 2].copy(), mod[:, 3].copy(), mod[:, 4].copy(), mod[:, 5].copy())
    h = _layernorm(x, axis=-1) * (1 + ca) + sa
    x = x + ga * _A_ref(h, A_wq, A_wk, A_wv, A_wo)
    h = _layernorm(x, axis=-1) * (1 + cb) + sb
    x = x + gb * _B_ref(h, B_w1, B_b1, B_w2, B_b2)
    return x

def setup_inputs():
    _inp = _fwd_setup_inputs()
    _gk = jax.random.fold_in(jax.random.key(int.from_bytes(__import__("os").urandom(4), "little")), 2 ** 31 - 1)
    _shapes = [[1, 2048, 512]]
    _dtypes = ['bfloat16']
    _gks = jax.random.split(_gk, len(_shapes))
    _gs = [jax.random.normal(k, s, dtype=jnp.dtype(d)) * 0.05 for k, s, d in zip(_gks, _shapes, _dtypes)]
    _inp['grad_out'] = _gs[0]
    return _inp

def reference(A_x, A_wq, A_wk, A_wv, A_wo, B_w1, B_b1, B_w2, B_b2, c, w_mod, B_x, grad_out):
    _const = dict(B_x=B_x)

    def _f(*_d):
        return _fwd_reference(**{'A_x': _d[0], 'A_wq': _d[1], 'A_wk': _d[2], 'A_wv': _d[3], 'A_wo': _d[4], 'B_w1': _d[5], 'B_b1': _d[6], 'B_w2': _d[7], 'B_b2': _d[8], 'c': _d[9], 'w_mod': _d[10], **_const})
    _out, _vjp = jax.vjp(_f, A_x, A_wq, A_wk, A_wv, A_wo, B_w1, B_b1, B_w2, B_b2, c, w_mod)
    _grads = _vjp(grad_out)
    _out0 = jnp.asarray(_out)
    return (_out0, *[jnp.asarray(_g) for _g in _grads])
```

```python
import jax
import jax.numpy as jnp
from jax import lax
import jax.experimental.pallas as pl
import jax.experimental.pallas.tpu as pltpu

S, D, F, H, DH = 2048, 512, 1376, 32, 16
f32, bf16 = jnp.float32, jnp.bfloat16
NT = (((1,), (1,)), ((), ()))
LOG2E = 1.4426950408889634
LN2 = 0.6931471805599453
QSCALE = 0.25 * LOG2E
EPS = 1e-5
GELU_C = 0.7978845608028654
GELU_A = 0.044715
L_MIN = 2.0 ** -30

QB = 512
NG = S // QB
CW = 512
NCH = S // CW
FCH = ((0, 512), (512, 1024), (1024, F))

NS = 11
N_H = 15
N_R = H - NS - N_H


def _plan():
    types = []
    early = min(N_H, NS + 4)
    types += ['H'] * early
    nh, nr = N_H - early, N_R
    while nh > 0 and nr > 0:
        types += ['R', 'H']
        nh -= 1
        nr -= 1
    types += ['H'] * nh + ['R'] * nr + ['V'] * NS
    assert len(types) == H
    slot = [0] * H
    hidx = [0] * H
    wait = [0] * H
    pending = [False] * NS
    nhh = 0
    nonr = [i for i in range(H) if types[i] != 'R']
    for i in range(H):
        nxt = min(k for k in nonr if k >= i)
        slot[i] = nonr.index(nxt) % NS
        wait[i] = int(pending[slot[i]])
        pending[slot[i]] = False
        if types[i] == 'H':
            hidx[i] = nhh
            nhh += 1
            pending[slot[i]] = True
    assert not any(pending)
    v_heads = [i for i in range(H) if types[i] == 'V']
    h_heads = [i for i in range(H) if types[i] == 'H']
    r_heads = [i for i in range(H) if types[i] == 'R']
    order = v_heads + h_heads
    bslot = [slot[i] for i in v_heads]
    for k in range(len(h_heads)):
        bslot.append(bslot[k])
    return types, slot, hidx, wait, order, bslot, r_heads


_TYPES, _SLOT, _HIDX, _WAIT, _BORDER, _BSLOT, _RHEADS = _plan()
N_ST = len(_BORDER)


def _gelu_and_grad(x):
    x2 = x * x
    t = jnp.tanh(GELU_C * x * (1.0 + GELU_A * x2))
    g = 0.5 * x * (1.0 + t)
    dg = 0.5 * (1.0 + t) + 0.5 * x * (1.0 - t * t) * (GELU_C * (1.0 + 3.0 * GELU_A * x2))
    return g, dg


def _ln_stats(x):
    mean = jnp.mean(x, axis=0, keepdims=True)
    xc = x - mean
    var = jnp.mean(xc * xc, axis=0, keepdims=True)
    return mean, lax.rsqrt(var + EPS)


def _ln_bwd(dxhat, xhat, rstd):
    m1 = jnp.mean(dxhat, axis=0, keepdims=True)
    m2 = jnp.mean(dxhat * xhat, axis=0, keepdims=True)
    return rstd * (dxhat - m1 - xhat * m2)


def _rowsum_T(x):
    acc = x[:, 0:128]
    for j in range(1, x.shape[1] // 128):
        acc = acc + x[:, j * 128:(j + 1) * 128]
    return jnp.sum(acc.T, axis=0, keepdims=True)


def _colsum(x):
    return jnp.sum(x, axis=0, keepdims=True)


def _rowsum_blk(x):
    return jnp.sum(x.T, axis=0, keepdims=True)


def _acc(a, t):
    return t if a is None else a + t


def _aug(v):
    hi = v.astype(bf16).astype(f32)
    r = v - hi
    mid = r.astype(bf16).astype(f32)
    lo = r - mid
    row = lax.broadcasted_iota(jnp.int32, (16, v.shape[1]), 0)
    out = jnp.where(row == 0, hi, jnp.where(row == 1, mid, jnp.where(row == 2, lo, 0.0)))
    return out.astype(bf16)


def _kernel(x_hbm, wq_hbm, wk_ref, wv_ref, wo_hbm, w1_hbm, b1_ref, w2_hbm, b2_ref, c_ref, wmod_hbm, g_hbm,
            out_hbm, dx_hbm, dwq_hbm, dwk_ref, dwv_ref, dwo_hbm, dw1_hbm, db1_ref, dw2_hbm, db2_ref, dc_ref,
            dwmod_hbm, spill_hbm,
            pc, q3, negm, oT3, aT, x1T, kva, kT, vat, l_s, st, modc, dmr, wqkv, wo_s, tbl, flag, psem):
    for i in range(H):
        tbl[0, i] = _SLOT[i]
        tbl[1, i] = _HIDX[i]
        tbl[2, i] = _WAIT[i]
        tbl[3, i] = int(_TYPES[i] == 'H')
    for i in range(N_ST):
        tbl[4, i] = _BORDER[i]
        tbl[5, i] = _BSLOT[i]
    for i in range(N_R):
        tbl[6, i] = _RHEADS[i]

    def col(j):
        return modc[:, j:j + 1]

    def chunk_cols(j):
        return slice(j * CW, (j + 1) * CW)

    def phase_a(w1, w2, gT, h2nT, sem_a):
        cp_wo = pltpu.make_async_copy(wo_hbm, wo_s, sem_a.at[3])
        cp_w1 = pltpu.make_async_copy(w1_hbm, w1, sem_a.at[4])
        cp_w2 = pltpu.make_async_copy(w2_hbm, w2, sem_a.at[5])

        def upto_stage3(xbuf, xT, wm1):
            cp_g = pltpu.make_async_copy(g_hbm, xbuf, sem_a.at[0])
            cp_wm1 = pltpu.make_async_copy(wmod_hbm.at[:, 2 * D:6 * D], wm1, sem_a.at[6])
            cf = c_ref[...].astype(f32)
            scb = (cf * jax.nn.sigmoid(cf)).astype(bf16)

            def stage1(wm0, wq_b, wqkvT, kvT, qn2):
                cp_wm0 = pltpu.make_async_copy(wmod_hbm.at[:, 0:2 * D], wm0, sem_a.at[1])
                cp_wq = pltpu.make_async_copy(wq_hbm, wq_b, sem_a.at[2])
                cp_xs = [pltpu.make_async_copy(x_hbm.at[chunk_cols(j), :], xbuf.at[chunk_cols(j), :], sem_a.at[7 + j])
                         for j in range(NCH)]
                cp_xs[0].start()
                cp_wm0.start()
                cp_wq.start()
                for cp in cp_xs[1:]:
                    cp.start()
                cp_wo.start()
                cp_wm1.start()
                for j in range(NCH):
                    cols = chunk_cols(j)
                    cp_xs[j].wait()
                    xb = xbuf[cols, :].T
                    xT[:, cols] = xb
                    xf = xb.astype(f32)
                    mean, rstd = _ln_stats(xf)
                    st[0:1, cols] = mean
                    st[1:2, cols] = rstd
                    x1T[:, cols] = (xf - mean) * rstd
                cp_wm0.wait()
                mod = jnp.dot(scb, wm0[...], preferred_element_type=f32)
                dmr[...] = jnp.zeros((8, D), f32)
                for j in range(2):
                    dmr[j:j + 1, :] = mod[:, j * D:(j + 1) * D]
                modc[...] = dmr[...].T
                cp_wq.wait()
                wq_v = wq_b[...]
                wkvT = jnp.concatenate([wk_ref[...], wv_ref[...], jnp.zeros((96, D), bf16)], axis=0)
                wqkv[:, 0:D] = wq_v
                wqkv[:, D:D + 128] = wkvT.T
                wqkvT[0:D, :] = wq_v.T
                wqkvT[D:D + 32, :] = wkvT[0:32, :]
                for j in range(NCH):
                    cols = chunk_cols(j)
                    h1b = (x1T[:, cols] * (1.0 + col(1)) + col(0)).astype(bf16)
                    qkv = jnp.dot(wqkvT[...], h1b, preferred_element_type=f32)
                    qs = (qkv[0:D] * QSCALE).astype(bf16)
                    q3[:, :, cols] = qs.reshape(H, DH, CW)
                    qf = qs.astype(f32)
                    qn2[:, cols] = jnp.sum((qf * qf).reshape(H, DH, CW), axis=1)
                    kvT[:, cols] = qkv[D:D + 32].astype(bf16)
                kt = kvT[0:16, :]
                vt = kvT[16:32, :]
                kT[0:16, :] = kt
                kT[16:32, :] = vt
                ones3 = (lax.broadcasted_iota(jnp.int32, (16, S), 0) < 3).astype(bf16)
                vat[0:16, :] = vt
                vat[16:32, :] = ones3
                kva[...] = jnp.concatenate([kt, ones3, vt], axis=0).T
                kf = kt.astype(f32)
                kmax2 = jnp.max(jnp.sum(kf * kf, axis=0, keepdims=True), axis=1, keepdims=True)
                negm[...] = -(jnp.sqrt(qn2[...] * kmax2) * (1.0 + 2.0 ** -10) + 2.0 ** -20)

            pl.run_scoped(stage1, pltpu.VMEM((D, 2 * D), bf16), pltpu.VMEM((D, D), bf16),
                          pltpu.VMEM((D + 32, D), bf16), pltpu.VMEM((32, S), bf16), pltpu.VMEM((H, S), f32))

            CK = 256
            NC = S // CK

            def head_fwd(h, slot):
                units = [(g, c) for g in range(NG) for c in range(NC)]
                ws = {}

                def stream(u):
                    g, c = units[u]
                    gc = slice(g * QB, (g + 1) * QB)
                    if g not in ws:
                        ws[g] = jnp.concatenate([q3[h, :, gc], _aug(negm[pl.ds(h, 1), gc])], axis=0)
                    ks = slice(c * CK, (c + 1) * CK)
                    s = jnp.dot(kva[ks, 0:32], ws[g], preferred_element_type=f32)
                    p = jnp.exp2(s)
                    pb = p.astype(bf16)
                    k0 = c * CK
                    pc[slot, k0 // QB, gc, (k0 % QB):(k0 % QB) + CK] = pb.T
                    return pb, jnp.sum(p.reshape(CK // 8, 8, QB), axis=0)

                cur = stream(0)
                lmin = None
                l8 = acc = None
                for u in range(len(units)):
                    g, c = units[u]
                    ks = slice(c * CK, (c + 1) * CK)
                    nxt = stream(u + 1) if u + 1 < len(units) else None
                    pb, ls = cur
                    pv = jnp.dot(kT[16:32, ks], pb, preferred_element_type=f32)
                    l8 = ls if c == 0 else l8 + ls
                    acc = pv if c == 0 else acc + pv
                    if c == NC - 1:
                        l = jnp.sum(l8, axis=0, keepdims=True)
                        oT3[h, :, g * QB:(g + 1) * QB] = (acc / l).astype(bf16)
                        l_s[pl.ds(h, 1), g * QB:(g + 1) * QB] = l
                        lmin = l if lmin is None else jnp.minimum(lmin, l)
                    cur = nxt
                return jnp.min(lmin)

            def true_max(h):
                def grp(g, _):
                    cols = pl.ds(pl.multiple_of(g * QB, QB), QB)
                    w = q3[h, :, cols]

                    def ch(c, m):
                        ks = pl.ds(pl.multiple_of(c * CK, CK), CK)
                        s = jnp.dot(kva[ks, 0:16], w, preferred_element_type=f32)
                        return jnp.maximum(m, jnp.max(s, axis=0, keepdims=True))

                    m = lax.fori_loop(0, NC, ch, jnp.full((1, QB), -jnp.inf, f32))
                    negm[pl.ds(h, 1), cols] = -m
                    return 0

                lax.fori_loop(0, NG, grp, 0)

            def spill_copy(slot, hi_):
                return pltpu.make_async_copy(pc.at[slot], spill_hbm.at[hi_], psem.at[slot])

            def fwd_step(h, _):
                slot = tbl[0, h]

                @pl.when(tbl[2, h] == 1)
                def _():
                    spill_copy(slot, 0).wait()

                @pl.when(h == H - 2)
                def _():
                    cp_g.start()
                    cp_w1.start()
                    cp_w2.start()

                flag[0] = 1

                def attempt(a, _):
                    @pl.when(flag[0] == 1)
                    def _():
                        @pl.when(a == 1)
                        def _():
                            true_max(h)

                        lmin = head_fwd(h, slot)
                        flag[0] = jnp.logical_not(lmin >= L_MIN).astype(jnp.int32)

                    return 0

                lax.fori_loop(0, 2, attempt, 0)

                @pl.when(tbl[3, h] == 1)
                def _():
                    spill_copy(slot, tbl[1, h]).start()

                return 0

            lax.fori_loop(0, H, fwd_step, 0)

            def stage3(woT):
                cp_wo.wait()
                cp_wm1.wait()
                woT[...] = wo_s[...].T
                mod = jnp.dot(scb, wm1[...], preferred_element_type=f32)
                for j in range(4):
                    dmr[2 + j:3 + j, :] = mod[:, j * D:(j + 1) * D]
                modc[...] = dmr[...].T
                for j in range(NCH):
                    cols = chunk_cols(j)
                    a = jnp.dot(woT[...], oT3[:, :, cols].reshape(D, CW), preferred_element_type=f32)
                    aT[:, cols] = a.astype(bf16)
                    x1 = xT[:, cols].astype(f32) + col(2) * a
                    x1T[:, cols] = x1
                    mean2, rstd2 = _ln_stats(x1)
                    h2 = ((x1 - mean2) * rstd2) * (1.0 + col(4)) + col(3)
                    mean3, rstd3 = _ln_stats(h2)
                    st[2:3, cols] = mean2
                    st[3:4, cols] = rstd2
                    st[4:5, cols] = mean3
                    st[5:6, cols] = rstd3
                    h2nT[:, cols] = ((h2 - mean3) * rstd3).astype(bf16)
                cp_g.wait()
                gT[...] = xbuf[...].T

            pl.run_scoped(stage3, pltpu.VMEM((D, D), bf16))

        pl.run_scoped(upto_stage3, pltpu.VMEM((S, D), bf16), pltpu.VMEM((D, S), bf16), pltpu.VMEM((D, 4 * D), bf16))

        def mlp(u_s, dgelu, dy_s, tT, stg2, sem2):
            dup_s = u_s
            cp_w1.wait()
            for f0, f1 in FCH:
                upre = (lax.dot_general(h2nT[...], w1[f0:f1, :], NT, preferred_element_type=f32)
                        + b1_ref[f0:f1].reshape(1, f1 - f0).astype(f32))
                uu, dgl = _gelu_and_grad(upre)
                u_s[:, f0:f1] = uu.astype(bf16)
                dgelu[:, f0:f1] = dgl.astype(bf16)
            cp_w2.wait()

            def out_copy(j):
                return pltpu.make_async_copy(stg2.at[j % 2, 0:CW, :], out_hbm.at[pl.ds(j * CW, CW), :], sem2.at[j % 2])

            dgb = None
            for j in range(NCH):
                cols = chunk_cols(j)
                y = jnp.dot(u_s[...], w2[:, cols], preferred_element_type=f32) + b2_ref[cols].reshape(1, CW).astype(f32)
                x2 = (x1T[:, cols] + col(5) * y).astype(bf16).T
                gf = gT[:, cols].astype(f32)
                t = _rowsum_T(gf * y)
                dgb = t if dgb is None else dgb + t
                dy = gf * col(5)
                db2_ref[cols] = jnp.sum(dy, axis=0).astype(bf16)
                dy_s[:, cols] = dy.astype(bf16)
                if j >= 2:
                    out_copy(j - 2).wait()
                stg2[j % 2, 0:CW, :] = x2
                out_copy(j).start()
            dmr[5:6, :] = dgb
            for j in range(NCH - 2, NCH):
                out_copy(j).wait()

            cps = []

            def dw_compute(rhs, idx):
                RB = F // 2
                j, jj = idx // NCH, idx % NCH
                return jnp.dot(tT[j * RB:(j + 1) * RB, :], rhs[:, chunk_cols(jj)],
                               preferred_element_type=f32).astype(bf16)

            def dw_emit(val, dst, idx):
                RB = F // 2
                j, jj = idx // NCH, idx % NCH
                k = len(cps)
                if k >= 2:
                    cps[k - 2].wait()
                stg2[k % 2] = val
                cp = pltpu.make_async_copy(stg2.at[k % 2], dst.at[j * RB:(j + 1) * RB, chunk_cols(jj)], sem2.at[k % 2])
                cp.start()
                cps.append(cp)

            tT[...] = u_s[...].T
            nxt_piece = 0
            for fi, (f0, f1) in enumerate(FCH):
                du = lax.dot_general(dy_s[...], w2[f0:f1, :], NT, preferred_element_type=f32)
                idxs = list(range(nxt_piece, nxt_piece + (3, 3, 2)[fi]))
                nxt_piece += len(idxs)
                v0 = dw_compute(dy_s, idxs[0])
                dup = du * dgelu[:, f0:f1].astype(f32)
                db1_ref[f0:f1] = jnp.sum(dup, axis=0).astype(bf16)
                dup_s[:, f0:f1] = dup.astype(bf16)
                dw_emit(v0, dw2_hbm, idxs[0])
                for idx in idxs[1:]:
                    dw_emit(dw_compute(dy_s, idx), dw2_hbm, idx)

            tT[...] = dup_s[...].T
            dga = dsb_ = dcb = None
            cb1 = jnp.broadcast_to(1.0 + col(4), (D, 128))
            sbc = jnp.broadcast_to(col(3), (D, 128))
            gac = jnp.broadcast_to(col(2), (D, 128))
            cb1_sum = _colsum(cb1)
            for j in range(NCH):
                cols = chunk_cols(j)
                dh2n = jnp.dot(dup_s[...], w1[:, cols], preferred_element_type=f32)
                v0 = dw_compute(h2nT, 2 * j)
                v1 = dw_compute(h2nT, 2 * j + 1)
                for bi in range(CW // 128):
                    bc = slice(j * CW + bi * 128, j * CW + (bi + 1) * 128)
                    g = dh2n[:, bi * 128:(bi + 1) * 128]
                    mean2, rstd2, mean3, rstd3 = st[2:3, bc], st[3:4, bc], st[4:5, bc], st[5:6, bc]
                    xh = (x1T[:, bc] - mean2) * rstd2
                    hn = (xh * cb1 + sbc - mean3) * rstd3
                    gc = g * cb1
                    hc = hn * cb1
                    m1 = _colsum(g) * (1.0 / D)
                    m2 = _colsum(g * hn) * (1.0 / D)
                    n1 = rstd3 * (_colsum(gc) - m1 * cb1_sum - m2 * _colsum(hc)) * (1.0 / D)
                    n2 = rstd3 * (_colsum(gc * xh) - m1 * _colsum(cb1 * xh) - m2 * _colsum(hc * xh)) * (1.0 / D)
                    xh = (x1T[:, bc] - mean2) * rstd2
                    hn = (xh * cb1 + sbc - mean3) * rstd3
                    dh2 = rstd3 * (g - m1 - hn * m2)
                    dx1 = gT[:, bc].astype(f32) + rstd2 * (dh2 * cb1 - n1 - xh * n2)
                    x1T[:, bc] = dx1
                    dga = _acc(dga, _rowsum_blk(dx1 * aT[:, bc].astype(f32)))
                    dsb_ = _acc(dsb_, _rowsum_blk(dh2))
                    dcb = _acc(dcb, _rowsum_blk(dh2 * xh))
                    aT[:, bc] = (dx1 * gac).astype(bf16)
                dw_emit(v0, dw1_hbm, 2 * j)
                dw_emit(v1, dw1_hbm, 2 * j + 1)
            dmr[2:3, :] = dga
            dmr[3:4, :] = dsb_
            dmr[4:5, :] = dcb
            for cp in cps[-2:]:
                cp.wait()

        pl.run_scoped(mlp, pltpu.VMEM((D, F), bf16), pltpu.VMEM((D, F), bf16), pltpu.VMEM((D, S), bf16),
                      pltpu.VMEM((F, D), bf16),
                      pltpu.VMEM((2, F // 2, CW), bf16), pltpu.SemaphoreType.DMA((2,)))

    pl.run_scoped(phase_a, pltpu.VMEM((F, S), bf16), pltpu.VMEM((F, S), bf16), pltpu.VMEM((D, S), bf16),
                  pltpu.VMEM((D, S), bf16), pltpu.SemaphoreType.DMA((7 + NCH,)))

    def phase_b(do3, negd, dq3, dqa, dkv, lhs, wmod, xbuf, stg, dwm, sem_b):
        cp_wmod = pltpu.make_async_copy(wmod_hbm, wmod, sem_b.at[0])
        cp_x = pltpu.make_async_copy(x_hbm, xbuf, sem_b.at[2])
        cp_wmod.start()
        cp_x.start()

        def load_copy(slot, hi_):
            return pltpu.make_async_copy(spill_hbm.at[hi_], pc.at[slot], psem.at[slot])

        cf = c_ref[...].astype(f32)
        sg = jax.nn.sigmoid(cf)
        sc_col = jnp.broadcast_to(cf * sg, (128, D)).T[:, 0:1]

        def mod_bwd(j):
            row = dmr[j:j + 1, :]
            dwm[:, j * D:(j + 1) * D] = (sc_col * row).astype(bf16)
            return lax.dot_general(row.astype(bf16), wmod[:, j * D:(j + 1) * D], NT, preferred_element_type=f32)

        dwo = lax.dot_general(oT3[...].reshape(D, S), aT[...], NT, preferred_element_type=f32)
        stg[...] = dwo.astype(bf16)
        cp_dwo = pltpu.make_async_copy(stg, dwo_hbm, sem_b.at[1])
        cp_dwo.start()
        for j in range(NCH):
            cols = chunk_cols(j)
            do = jnp.dot(wo_s[...], aT[:, cols], preferred_element_type=f32).reshape(H, DH, CW)
            linv = 1.0 / l_s[:, cols]
            dob = (do * linv.reshape(H, 1, CW)).astype(bf16)
            do3[:, :, cols] = dob
            negd[:, cols] = -jnp.sum(dob.astype(f32) * oT3[:, :, cols].astype(f32), axis=1)
        dkv[...] = jnp.zeros((32, S), f32)
        cp_wmod.wait()
        dsc = mod_bwd(2) + mod_bwd(3) + mod_bwd(4) + mod_bwd(5)
        dmr[6:7, :] = dsc
        cp_dwm1 = pltpu.make_async_copy(dwm.at[:, 2 * D:6 * D], dwmod_hbm.at[:, 2 * D:6 * D], sem_b.at[3])
        cp_dwm1.start()

        def head_bwd_stored(h, slot):
            QC, NP = 256, 2
            PC = QC // NP
            NQC = S // QC
            lhs[...] = jnp.concatenate([do3[h], _aug(negd[pl.ds(h, 1), :])], axis=0).T
            units = [(qc, g) for qc in range(NQC) for g in range(NG)]

            def piece(u, pi):
                qc, g = units[u]
                r0 = qc * QC + pi * PC
                rows = slice(r0, r0 + PC)
                dp = jnp.dot(lhs[rows, :], vat[:, g * QB:(g + 1) * QB], preferred_element_type=f32)
                return (pc[slot, g, rows, :].astype(f32) * dp).astype(bf16)

            cur = [piece(0, pi) for pi in range(NP)]
            for u in range(len(units)):
                qc, g = units[u]
                qs = slice(qc * QC, (qc + 1) * QC)
                gs = slice(g * QB, (g + 1) * QB)
                dsb = jnp.concatenate(cur, axis=0)
                nxt = []
                for pi in range(NP):
                    if u + 1 < len(units):
                        nxt.append(piece(u + 1, pi))
                    if pi == 0:
                        dkv[16:32, gs] += jnp.dot(do3[h, :, qs], pc[slot, g, qs, :], preferred_element_type=f32)
                    else:
                        t = lax.dot_general(kT[0:16, gs], dsb, NT, preferred_element_type=f32)
                        if g == 0:
                            dqa[:, qs] = t
                        else:
                            dqa[:, qs] += t
                        dkv[0:16, gs] += jnp.dot(q3[h, :, qs], dsb, preferred_element_type=f32)
                cur = nxt
            dq3[h] = (dqa[...] * 0.25).astype(bf16)

        def head_bwd_rec(h):
            CK, NP = 128, 2
            NC = S // CK
            PC = CK // NP
            units = [(g, c) for g in range(NG) for c in range(NC)]
            ws = {}

            def piece(u, pi):
                g, c = units[u]
                gc = slice(g * QB, (g + 1) * QB)
                if g not in ws:
                    z = jnp.zeros((16, QB), bf16)
                    ws[g] = jnp.concatenate([
                        jnp.concatenate([q3[h, :, gc], z], axis=1),
                        jnp.concatenate([_aug(negm[pl.ds(h, 1), gc]), _aug(negd[pl.ds(h, 1), gc])], axis=1),
                        jnp.concatenate([z, do3[h, :, gc]], axis=1)], axis=0)
                r0 = c * CK + pi * PC
                o = jnp.dot(kva[r0:r0 + PC, :], ws[g], preferred_element_type=f32)
                p = jnp.exp2(o[:, :QB])
                ds = p * o[:, QB:]
                return p.astype(bf16), ds.astype(bf16)

            cur = [piece(0, pi) for pi in range(NP)]
            dq = None
            for u in range(len(units)):
                g, c = units[u]
                gc = slice(g * QB, (g + 1) * QB)
                ks = slice(c * CK, (c + 1) * CK)
                dsb = jnp.concatenate([t[1] for t in cur], axis=0)
                pb = jnp.concatenate([t[0] for t in cur], axis=0)
                nxt = []
                for pi in range(NP):
                    if u + 1 < len(units):
                        nxt.append(piece(u + 1, pi))
                    if pi == 0:
                        dkv[16:32, ks] += lax.dot_general(do3[h, :, gc], pb, NT, preferred_element_type=f32)
                    else:
                        t = jnp.dot(kT[0:16, ks], dsb, preferred_element_type=f32)
                        dq = t if c == 0 else dq + t
                        dkv[0:16, ks] += lax.dot_general(q3[h, :, gc], dsb, NT, preferred_element_type=f32)
                if c == NC - 1:
                    dq3[h, :, gc] = (dq * 0.25).astype(bf16)
                cur = nxt

        def bwd_stored_step(i, _):
            h = tbl[4, i]
            slot = tbl[5, i]

            @pl.when(i >= NS)
            def _():
                load_copy(slot, 0).wait()

            head_bwd_stored(h, slot)

            @pl.when(i < N_H)
            def _():
                load_copy(slot, i).start()

            return 0

        lax.fori_loop(0, N_ST, bwd_stored_step, 0)

        if N_R > 0:
            def bwd_rec_step(i, _):
                head_bwd_rec(tbl[6, i])
                return 0

            lax.fori_loop(0, N_R, bwd_rec_step, 0)

        def stage8(xT, dkvb, xstg, sem8):
            cp_x.wait()
            cp_dwo.wait()
            xT[...] = xbuf[...].T
            dkvb[0:16, :] = (dkv[0:16, :] * LN2).astype(bf16)
            dkvb[16:32, :] = dkv[16:32, :].astype(bf16)
            dkvb[32:128, :] = jnp.zeros((96, S), bf16)

            def dx_copy(j):
                return pltpu.make_async_copy(xstg.at[j % 2], dx_hbm.at[pl.ds(j * CW, CW), :], sem8.at[1 + j % 2])

            dsa = dca = dw = dwkvT = None
            ca1 = jnp.broadcast_to(1.0 + col(1), (D, 128))
            for j in range(NCH):
                cols = chunk_cols(j)
                dqc = dq3[:, :, cols].reshape(D, CW)
                dh1 = (jnp.dot(wqkv[:, 0:D], dqc, preferred_element_type=f32)
                       + jnp.dot(wqkv[:, D:D + 128], dkvb[:, cols], preferred_element_type=f32))
                h1b = ((xT[:, cols].astype(f32) - st[0:1, cols]) * st[1:2, cols] * (1.0 + col(1))
                       + col(0)).astype(bf16)
                t = lax.dot_general(h1b, dqc, NT, preferred_element_type=f32)
                dw = t if dw is None else dw + t
                t = lax.dot_general(dkvb[0:32, cols], h1b, NT, preferred_element_type=f32)
                dwkvT = t if dwkvT is None else dwkvT + t
                dxs = []
                for bi in range(CW // 128):
                    bc = slice(j * CW + bi * 128, j * CW + (bi + 1) * 128)
                    g = dh1[:, bi * 128:(bi + 1) * 128]
                    mean1, rstd1 = st[0:1, bc], st[1:2, bc]
                    xh = (xT[:, bc].astype(f32) - mean1) * rstd1
                    gx = g * xh
                    m1 = _colsum(g * ca1) * (1.0 / D)
                    m2 = _colsum(gx * ca1) * (1.0 / D)
                    dsa = _acc(dsa, _rowsum_blk(g))
                    dca = _acc(dca, _rowsum_blk(gx))
                    xh = (xT[:, bc].astype(f32) - mean1) * rstd1
                    dxs.append((x1T[:, bc] + rstd1 * (g * ca1 - m1 - xh * m2)).astype(bf16).T)
                dx = jnp.concatenate(dxs, axis=0)
                if j >= 2:
                    dx_copy(j - 2).wait()
                xstg[j % 2] = dx
                dx_copy(j).start()
            stg[...] = dw.astype(bf16)
            cp_dwq = pltpu.make_async_copy(stg, dwq_hbm, sem8.at[0])
            cp_dwq.start()
            dwk_ref[...] = dwkvT[0:16].astype(bf16)
            dwv_ref[...] = dwkvT[16:32].astype(bf16)
            dmr[0:1, :] = dsa
            dmr[1:2, :] = dca
            dsc2 = dmr[6:7, :] + mod_bwd(0) + mod_bwd(1)
            cp_dwm0 = pltpu.make_async_copy(dwm.at[:, 0:2 * D], dwmod_hbm.at[:, 0:2 * D], sem_b.at[4])
            cp_dwm0.start()
            dc_ref[...] = (dsc2 * (sg * (1.0 + cf * (1.0 - sg)))).astype(bf16)
            for j in range(NCH - 2, NCH):
                dx_copy(j).wait()
            cp_dwm1.wait()
            cp_dwm0.wait()
            cp_dwq.wait()

        pl.run_scoped(stage8, pltpu.VMEM((D, S), bf16), pltpu.VMEM((128, S), bf16),
                      pltpu.VMEM((2, CW, D), bf16), pltpu.SemaphoreType.DMA((3,)))

    pl.run_scoped(phase_b, pltpu.VMEM((H, DH, S), bf16), pltpu.VMEM((H, S), f32), pltpu.VMEM((H, DH, S), bf16),
                  pltpu.VMEM((DH, S), f32), pltpu.VMEM((32, S), f32), pltpu.VMEM((S, 32), bf16),
                  pltpu.VMEM((D, 6 * D), bf16), pltpu.VMEM((S, D), bf16), pltpu.VMEM((D, D), bf16),
                  pltpu.VMEM((D, 6 * D), bf16), pltpu.SemaphoreType.DMA((5,)))


@jax.jit
def pallas_adaLN_cond__grouped_kv_mqa__mixer_token_mlp__prompt_kernel(
    A_x: jax.Array,
    A_wq: jax.Array,
    A_wk: jax.Array,
    A_wv: jax.Array,
    A_wo: jax.Array,
    B_x: jax.Array,
    B_w1: jax.Array,
    B_b1: jax.Array,
    B_w2: jax.Array,
    B_b2: jax.Array,
    c: jax.Array,
    w_mod: jax.Array,
    grad_out: jax.Array,
):
    any_spec = pl.BlockSpec(memory_space=pl.ANY)
    vmem_spec = pl.BlockSpec(memory_space=pltpu.VMEM)
    sds = jax.ShapeDtypeStruct
    out_shape = (
        sds((S, D), bf16), sds((S, D), bf16), sds((D, D), bf16), sds((DH, D), bf16), sds((DH, D), bf16),
        sds((D, D), bf16), sds((F, S), bf16), sds((F,), bf16), sds((F, S), bf16), sds((S,), bf16),
        sds((1, D), bf16), sds((D, 6 * D), bf16), sds((N_H, NG, S, QB), bf16),
    )
    out_specs = (any_spec, any_spec, any_spec, vmem_spec, vmem_spec, any_spec, any_spec, vmem_spec, any_spec,
                 vmem_spec, vmem_spec, any_spec, any_spec)
    in_specs = [any_spec, any_spec, vmem_spec, vmem_spec, any_spec, any_spec, vmem_spec, any_spec, vmem_spec,
                vmem_spec, any_spec, any_spec]
    scratch = [
        pltpu.VMEM((NS, NG, S, QB), bf16),
        pltpu.VMEM((H, DH, S), bf16),
        pltpu.VMEM((H, S), f32),
        pltpu.VMEM((H, DH, S), bf16),
        pltpu.VMEM((D, S), bf16),
        pltpu.VMEM((D, S), f32),
        pltpu.VMEM((S, 48), bf16),
        pltpu.VMEM((32, S), bf16),
        pltpu.VMEM((32, S), bf16),
        pltpu.VMEM((H, S), f32),
        pltpu.VMEM((8, S), f32),
        pltpu.VMEM((D, 8), f32),
        pltpu.VMEM((8, D), f32),
        pltpu.VMEM((D, D + 128), bf16),
        pltpu.VMEM((D, D), bf16),
        pltpu.SMEM((8, H), jnp.int32),
        pltpu.SMEM((1,), jnp.int32),
        pltpu.SemaphoreType.DMA((NS,)),
    ]
    outs = pl.pallas_call(
        _kernel,
        out_shape=out_shape,
        in_specs=in_specs,
        out_specs=out_specs,
        scratch_shapes=scratch,
        compiler_params=pltpu.CompilerParams(vmem_limit_bytes=128 * 2 ** 20),
    )(A_x.reshape(S, D), A_wq, A_wk.T, A_wv.T, A_wo, B_w1.T, B_b1, B_w2, B_b2, c, w_mod,
      grad_out.reshape(S, D))
    (out, dx, dwq, dwk, dwv, dwo, dw1, db1, dw2, db2, dc, dwmod, _) = outs
    return (out.reshape(1, S, D), dx.reshape(1, S, D), dwq, dwk.T, dwv.T, dwo, dw1.T, db1, dw2, db2, dc, dwmod)
```

```python
import jax
import jax.numpy as jnp
from jax import lax
import jax.experimental.pallas as pl
import jax.experimental.pallas.tpu as pltpu

S, D, F, H, DH = 2048, 512, 1376, 32, 16
f32, bf16 = jnp.float32, jnp.bfloat16
NT = (((1,), (1,)), ((), ()))
LOG2E = 1.4426950408889634
LN2 = 0.6931471805599453
QSCALE = 0.25 * LOG2E
EPS = 1e-5
GELU_C = 0.7978845608028654
GELU_A = 0.044715
L_MIN = 2.0 ** -30

QB = 512
NG = S // QB
CW = 512
NCH = S // CW
FCH = ((0, 512), (512, 1024), (1024, F))

NS = 11
XS = NS
N_H = 15
N_R = H - NS - N_H - 1
X_HEAD = N_H


def _plan():
    types = ['H'] * N_H + ['X'] + ['R'] * N_R + ['V'] * NS
    assert len(types) == H
    slot = [0] * H
    hidx = [0] * H
    wait = [0] * H
    pending = [False] * NS
    nhh = 0
    rot = [i for i in range(H) if types[i] in 'HV']
    for i in range(H):
        if types[i] == 'X':
            slot[i] = XS
            continue
        nxt = min(k for k in rot if k >= i)
        slot[i] = rot.index(nxt) % NS
        wait[i] = int(pending[slot[i]])
        pending[slot[i]] = False
        if types[i] == 'H':
            hidx[i] = nhh
            nhh += 1
            pending[slot[i]] = True
    assert not any(pending)
    v_heads = [i for i in range(H) if types[i] == 'V']
    h_heads = [i for i in range(H) if types[i] == 'H']
    r_heads = [i for i in range(H) if types[i] == 'R']
    order = v_heads + [X_HEAD] + h_heads
    bslot = [slot[i] for i in v_heads] + [XS]
    for k in range(len(h_heads)):
        bslot.append(bslot[k])
    return types, slot, hidx, wait, order, bslot, r_heads


_TYPES, _SLOT, _HIDX, _WAIT, _BORDER, _BSLOT, _RHEADS = _plan()
N_ST = len(_BORDER)


def _gelu_and_grad(x):
    x2 = x * x
    t = jnp.tanh(GELU_C * x * (1.0 + GELU_A * x2))
    g = 0.5 * x * (1.0 + t)
    dg = 0.5 * (1.0 + t) + 0.5 * x * (1.0 - t * t) * (GELU_C * (1.0 + 3.0 * GELU_A * x2))
    return g, dg


def _ln_stats(x):
    mean = jnp.mean(x, axis=0, keepdims=True)
    xc = x - mean
    var = jnp.mean(xc * xc, axis=0, keepdims=True)
    return mean, lax.rsqrt(var + EPS)


def _rowsum_T(x):
    acc = x[:, 0:128]
    for j in range(1, x.shape[1] // 128):
        acc = acc + x[:, j * 128:(j + 1) * 128]
    return jnp.sum(acc.T, axis=0, keepdims=True)


def _colsum(x):
    return jnp.sum(x, axis=0, keepdims=True)


def _rowsum_blk(x):
    return jnp.sum(x.T, axis=0, keepdims=True)


def _acc(a, t):
    return t if a is None else a + t


def _aug(v):
    hi = v.astype(bf16).astype(f32)
    r = v - hi
    mid = r.astype(bf16).astype(f32)
    lo = r - mid
    row = lax.broadcasted_iota(jnp.int32, (16, v.shape[1]), 0)
    out = jnp.where(row == 0, hi, jnp.where(row == 1, mid, jnp.where(row == 2, lo, 0.0)))
    return out.astype(bf16)


def _kernel(x_hbm, wq_hbm, wk_ref, wv_ref, wo_hbm, w1_hbm, b1_ref, w2_hbm, b2_ref, c_ref, wmod_hbm, g_hbm,
            out_hbm, dx_hbm, dwq_hbm, dwk_ref, dwv_ref, dwo_hbm, dw1_hbm, db1_ref, dw2_hbm, db2_ref, dc_ref,
            dwmod_hbm, spill_hbm,
            pc, q3, negm, oT3, aT, x1T, kva, kT, vat, l_s, st, modc, dmr, wo_s, tbl, flag, psem, msem, stg2, sem2):
    for i in range(H):
        tbl[0, i] = _SLOT[i]
        tbl[1, i] = _HIDX[i]
        tbl[2, i] = _WAIT[i]
        tbl[3, i] = int(_TYPES[i] == 'H')
    for i in range(N_ST):
        tbl[4, i] = _BORDER[i]
        tbl[5, i] = _BSLOT[i]
    for i in range(N_R):
        tbl[6, i] = _RHEADS[i]

    def col(j):
        return modc[:, j:j + 1]

    def chunk_cols(j):
        return slice(j * CW, (j + 1) * CW)

    def blk(slot, g, r):
        return pc.at[slot, g, r * D:(r + 1) * D, :]

    def wm_copy(j, slot, sem):
        return pltpu.make_async_copy(wmod_hbm.at[:, j * D:(j + 1) * D], blk(slot, 0, j % 4), sem)

    def phase_a(w1, gT, h2nT, sem_a):
        cp_wo = pltpu.make_async_copy(wo_hbm, wo_s, sem_a.at[3])
        cp_w1 = [pltpu.make_async_copy(w1_hbm.at[f0:f1, :], w1.at[f0:f1, :], sem_a.at[(0, 4, 5)[i]])
                 for i, (f0, f1) in enumerate(FCH)]
        cp_w2 = [pltpu.make_async_copy(w2_hbm.at[:, chunk_cols(j)], pc.at[XS, j, 0:F, :], sem_a.at[7 + NCH + j])
                 for j in range(NCH)]

        def upto_stage3(xT, wm1):
            cp_wm1 = pltpu.make_async_copy(wmod_hbm.at[:, 2 * D:6 * D], wm1, sem_a.at[6])
            cf = c_ref[...].astype(f32)
            scb = (cf * jax.nn.sigmoid(cf)).astype(bf16)

            def stage1(wm0, wq_b, wqkvT, kvT, qn2):
                xbuf = pc.at[0, 0]
                cp_wm0 = pltpu.make_async_copy(wmod_hbm.at[:, 0:2 * D], wm0, sem_a.at[1])
                cp_wq = pltpu.make_async_copy(wq_hbm, wq_b, sem_a.at[2])
                cp_xs = [pltpu.make_async_copy(x_hbm.at[chunk_cols(j), :], xbuf.at[chunk_cols(j), :], sem_a.at[7 + j])
                         for j in range(NCH)]
                cp_xs[0].start()
                cp_wm0.start()
                cp_wq.start()
                for cp in cp_xs[1:]:
                    cp.start()
                def ln1_chunk(j):
                    cols = chunk_cols(j)
                    xb = xbuf[cols, :].T
                    xT[:, cols] = xb
                    for bi in range(CW // 128):
                        bc = slice(j * CW + bi * 128, j * CW + (bi + 1) * 128)
                        mean = _colsum(xT[:, bc].astype(f32)) * (1.0 / D)
                        xc = xT[:, bc].astype(f32) - mean
                        st[0:1, bc] = mean
                        st[1:2, bc] = lax.rsqrt(_colsum(xc * xc) * (1.0 / D) + EPS)

                cp_xs[0].wait()
                ln1_chunk(0)
                cp_wm0.wait()
                mod = jnp.dot(scb, wm0[...], preferred_element_type=f32)
                dmr[...] = jnp.zeros((8, D), f32)
                for j in range(2):
                    dmr[j:j + 1, :] = mod[:, j * D:(j + 1) * D]
                modc[...] = dmr[...].T
                cp_wq.wait()
                wq_v = wq_b[...]
                wkvT = jnp.concatenate([wk_ref[...], wv_ref[...], jnp.zeros((96, D), bf16)], axis=0)
                wqkvT[0:D, :] = wq_v.T
                wqkvT[D:D + 32, :] = wkvT[0:32, :]
                cp_xs[1].wait()
                for j in range(NCH):
                    cols = chunk_cols(j)
                    h1b = ((xT[:, cols].astype(f32) - st[0:1, cols]) * st[1:2, cols] * (1.0 + col(1))
                           + col(0)).astype(bf16)
                    qkv = jnp.dot(wqkvT[...], h1b, preferred_element_type=f32)
                    if j + 1 < NCH:
                        ln1_chunk(j + 1)
                    qs = (qkv[0:D] * QSCALE).astype(bf16)
                    q3[:, :, cols] = qs.reshape(H, DH, CW)
                    qf = qs.astype(f32)
                    qn2[:, cols] = jnp.sum((qf * qf).reshape(H, DH, CW), axis=1)
                    kvT[:, cols] = qkv[D:D + 32].astype(bf16)
                    if j + 2 < NCH:
                        cp_xs[j + 2].wait()
                cp_wo.start()
                cp_wm1.start()
                kt = kvT[0:16, :]
                vt = kvT[16:32, :]
                kT[0:16, :] = kt
                kT[16:32, :] = vt
                ones3 = (lax.broadcasted_iota(jnp.int32, (16, S), 0) < 3).astype(bf16)
                vat[0:16, :] = vt
                vat[16:32, :] = ones3
                kva[...] = jnp.concatenate([kt, ones3, vt], axis=0).T
                kf = kt.astype(f32)
                kmax2 = jnp.max(jnp.sum(kf * kf, axis=0, keepdims=True), axis=1, keepdims=True)
                negm[...] = -(jnp.sqrt(qn2[...] * kmax2) * (1.0 + 2.0 ** -10) + 2.0 ** -20)

            pl.run_scoped(stage1, pltpu.VMEM((D, 2 * D), bf16), pltpu.VMEM((D, D), bf16),
                          pltpu.VMEM((D + 32, D), bf16), pltpu.VMEM((32, S), bf16), pltpu.VMEM((H, S), f32))

            CK = 256
            NC = S // CK

            def head_fwd(h, slot):
                units = [(g, c) for g in range(NG) for c in range(NC)]
                ws = {}

                def stream(u):
                    g, c = units[u]
                    gc = slice(g * QB, (g + 1) * QB)
                    if g not in ws:
                        ws[g] = jnp.concatenate([q3[h, :, gc], _aug(negm[pl.ds(h, 1), gc])], axis=0)
                    ks = slice(c * CK, (c + 1) * CK)
                    s = jnp.dot(kva[ks, 0:32], ws[g], preferred_element_type=f32)
                    p = jnp.exp2(s)
                    pb = p.astype(bf16)
                    k0 = c * CK
                    pc[slot, k0 // QB, gc, (k0 % QB):(k0 % QB) + CK] = pb.T
                    return pb, jnp.sum(p.reshape(CK // 8, 8, QB), axis=0)

                cur = stream(0)
                lmin = None
                l8 = acc = None
                for u in range(len(units)):
                    g, c = units[u]
                    ks = slice(c * CK, (c + 1) * CK)
                    nxt = stream(u + 1) if u + 1 < len(units) else None
                    pb, ls = cur
                    pv = jnp.dot(kT[16:32, ks], pb, preferred_element_type=f32)
                    l8 = ls if c == 0 else l8 + ls
                    acc = pv if c == 0 else acc + pv
                    if c == NC - 1:
                        l = jnp.sum(l8, axis=0, keepdims=True)
                        oT3[h, :, g * QB:(g + 1) * QB] = (acc / l).astype(bf16)
                        l_s[pl.ds(h, 1), g * QB:(g + 1) * QB] = l
                        lmin = l if lmin is None else jnp.minimum(lmin, l)
                    cur = nxt
                return jnp.min(lmin)

            def true_max(h):
                def grp(g, _):
                    cols = pl.ds(pl.multiple_of(g * QB, QB), QB)
                    w = q3[h, :, cols]

                    def ch(c, m):
                        ks = pl.ds(pl.multiple_of(c * CK, CK), CK)
                        s = jnp.dot(kva[ks, 0:16], w, preferred_element_type=f32)
                        return jnp.maximum(m, jnp.max(s, axis=0, keepdims=True))

                    m = lax.fori_loop(0, NC, ch, jnp.full((1, QB), -jnp.inf, f32))
                    negm[pl.ds(h, 1), cols] = -m
                    return 0

                lax.fori_loop(0, NG, grp, 0)

            def spill_copy(slot, hi_):
                return pltpu.make_async_copy(pc.at[slot], spill_hbm.at[hi_], psem.at[slot])

            def fwd_step(h, _):
                slot = tbl[0, h]

                @pl.when(tbl[2, h] == 1)
                def _():
                    spill_copy(slot, 0).wait()

                @pl.when(h == H - 2)
                def _():
                    for cp in cp_w1:
                        cp.start()

                @pl.when(h == H - 1)
                def _():
                    spill_copy(XS, N_H).start()

                flag[0] = 1

                def attempt(a, _):
                    @pl.when(flag[0] == 1)
                    def _():
                        @pl.when(a == 1)
                        def _():
                            true_max(h)

                        lmin = head_fwd(h, slot)
                        flag[0] = jnp.logical_not(lmin >= L_MIN).astype(jnp.int32)

                    return 0

                lax.fori_loop(0, 2, attempt, 0)

                @pl.when(tbl[3, h] == 1)
                def _():
                    spill_copy(slot, tbl[1, h]).start()

                return 0

            lax.fori_loop(0, H, fwd_step, 0)

            def stage3(woT):
                cp_wo.wait()
                cp_wm1.wait()
                woT[...] = wo_s[...].T
                mod = jnp.dot(scb, wm1[...], preferred_element_type=f32)
                for j in range(4):
                    dmr[2 + j:3 + j, :] = mod[:, j * D:(j + 1) * D]
                modc[...] = dmr[...].T
                for j in range(NCH):
                    cols = chunk_cols(j)
                    a = jnp.dot(woT[...], oT3[:, :, cols].reshape(D, CW), preferred_element_type=f32)
                    aT[:, cols] = a.astype(bf16)
                    x1 = xT[:, cols].astype(f32) + col(2) * a
                    x1T[:, cols] = x1
                    mean2, rstd2 = _ln_stats(x1)
                    h2 = ((x1 - mean2) * rstd2) * (1.0 + col(4)) + col(3)
                    mean3, rstd3 = _ln_stats(h2)
                    st[2:3, cols] = mean2
                    st[3:4, cols] = rstd2
                    st[4:5, cols] = mean3
                    st[5:6, cols] = rstd3
                    h2nT[:, cols] = ((h2 - mean3) * rstd3).astype(bf16)

            pl.run_scoped(stage3, pltpu.VMEM((D, D), bf16))

        pl.run_scoped(upto_stage3, pltpu.VMEM((D, S), bf16), pltpu.VMEM((D, 4 * D), bf16))

        def mlp(u_s, dgelu, tT, gsem):
            dup_s = u_s

            def dy_blk(j):
                return pc.at[XS, j, F:F + D, :]
            def g_copy(j):
                return pltpu.make_async_copy(g_hbm.at[chunk_cols(j), :], tT.at[chunk_cols(j % 2), :], gsem.at[j % 2])

            g_copy(0).start()
            g_copy(1).start()
            for fi, (f0, f1) in enumerate(FCH):
                cp_w1[fi].wait()
                upre = (lax.dot_general(h2nT[...], w1[f0:f1, :], NT, preferred_element_type=f32)
                        + b1_ref[f0:f1].reshape(1, f1 - f0).astype(f32))
                uu, dgl = _gelu_and_grad(upre)
                u_s[:, f0:f1] = uu.astype(bf16)
                dgelu[:, f0:f1] = dgl.astype(bf16)
                if fi == 1:
                    pltpu.make_async_copy(pc.at[XS], spill_hbm.at[N_H], psem.at[XS]).wait()
                    for cp in cp_w2:
                        cp.start()

            def out_copy(j):
                return pltpu.make_async_copy(stg2.at[j % 2, 0:CW, :], out_hbm.at[pl.ds(j * CW, CW), :], sem2.at[j % 2])

            dgb = None
            for j in range(NCH):
                cols = chunk_cols(j)
                cp_w2[j].wait()
                g_copy(j).wait()
                gb = tT[chunk_cols(j % 2), :].T
                gT[:, cols] = gb
                y = jnp.dot(u_s[...], pc[XS, j, 0:F, :], preferred_element_type=f32) + b2_ref[cols].reshape(1, CW).astype(f32)
                x2 = (x1T[:, cols] + col(5) * y).astype(bf16).T
                gf = gb.astype(f32)
                t = _rowsum_T(gf * y)
                dgb = t if dgb is None else dgb + t
                dy = gf * col(5)
                db2_ref[cols] = jnp.sum(dy, axis=0).astype(bf16)
                dy_blk(j)[...] = dy.astype(bf16)
                if j >= 2:
                    out_copy(j - 2).wait()
                stg2[j % 2, 0:CW, :] = x2
                out_copy(j).start()
                if j + 2 < NCH:
                    g_copy(j + 2).start()
            dmr[5:6, :] = dgb

            cps = [out_copy(NCH - 2), out_copy(NCH - 1)]

            def dy_rhs(jj):
                return dy_blk(jj)[...]

            def h2n_rhs(jj):
                return h2nT[:, chunk_cols(jj)]

            def dw_compute(rhs, idx):
                RB = F // 2
                j, jj = idx // NCH, idx % NCH
                return jnp.dot(tT[j * RB:(j + 1) * RB, :], rhs(jj), preferred_element_type=f32).astype(bf16)

            def dw_emit(val, dst, idx):
                RB = F // 2
                j, jj = idx // NCH, idx % NCH
                k = len(cps)
                if k >= 2:
                    cps[k - 2].wait()
                stg2[k % 2] = val
                cp = pltpu.make_async_copy(stg2.at[k % 2], dst.at[j * RB:(j + 1) * RB, chunk_cols(jj)], sem2.at[k % 2])
                cp.start()
                cps.append(cp)

            tT[...] = u_s[...].T
            nxt_piece = 0
            for fi, (f0, f1) in enumerate(FCH):
                du = None
                for jj in range(NCH):
                    du = _acc(du, lax.dot_general(dy_blk(jj)[...], pc[XS, jj, f0:f1, :], NT,
                                                  preferred_element_type=f32))
                idxs = list(range(nxt_piece, nxt_piece + (3, 3, 2)[fi]))
                nxt_piece += len(idxs)
                v0 = dw_compute(dy_rhs, idxs[0])
                dup = du * dgelu[:, f0:f1].astype(f32)
                db1_ref[f0:f1] = jnp.sum(dup, axis=0).astype(bf16)
                dup_s[:, f0:f1] = dup.astype(bf16)
                dw_emit(v0, dw2_hbm, idxs[0])
                for idx in idxs[1:]:
                    dw_emit(dw_compute(dy_rhs, idx), dw2_hbm, idx)

            for j in range(2, 6):
                wm_copy(j, XS, msem.at[j]).start()
            tT[...] = dup_s[...].T
            dga = dsb_ = dcb = None
            cb1 = jnp.broadcast_to(1.0 + col(4), (D, 128))
            sbc = jnp.broadcast_to(col(3), (D, 128))
            gac = jnp.broadcast_to(col(2), (D, 128))
            cb1_sum = _colsum(cb1)
            for j in range(NCH):
                cols = chunk_cols(j)
                dh2n = jnp.dot(dup_s[...], w1[:, cols], preferred_element_type=f32)
                v0 = dw_compute(h2n_rhs, 2 * j)
                v1 = dw_compute(h2n_rhs, 2 * j + 1)
                for bi in range(CW // 128):
                    bc = slice(j * CW + bi * 128, j * CW + (bi + 1) * 128)
                    g = dh2n[:, bi * 128:(bi + 1) * 128]
                    mean2, rstd2, mean3, rstd3 = st[2:3, bc], st[3:4, bc], st[4:5, bc], st[5:6, bc]
                    xh = (x1T[:, bc] - mean2) * rstd2
                    hn = (xh * cb1 + sbc - mean3) * rstd3
                    gc = g * cb1
                    hc = hn * cb1
                    m1 = _colsum(g) * (1.0 / D)
                    m2 = _colsum(g * hn) * (1.0 / D)
                    n1 = rstd3 * (_colsum(gc) - m1 * cb1_sum - m2 * _colsum(hc)) * (1.0 / D)
                    n2 = rstd3 * (_colsum(gc * xh) - m1 * _colsum(cb1 * xh) - m2 * _colsum(hc * xh)) * (1.0 / D)
                    xh = (x1T[:, bc] - mean2) * rstd2
                    hn = (xh * cb1 + sbc - mean3) * rstd3
                    dh2 = rstd3 * (g - m1 - hn * m2)
                    dx1 = gT[:, bc].astype(f32) + rstd2 * (dh2 * cb1 - n1 - xh * n2)
                    x1T[:, bc] = dx1
                    dga = _acc(dga, _rowsum_blk(dx1 * aT[:, bc].astype(f32)))
                    dsb_ = _acc(dsb_, _rowsum_blk(dh2))
                    dcb = _acc(dcb, _rowsum_blk(dh2 * xh))
                    aT[:, bc] = (dx1 * gac).astype(bf16)
                dw_emit(v0, dw1_hbm, 2 * j)
                dw_emit(v1, dw1_hbm, 2 * j + 1)
            dmr[2:3, :] = dga
            dmr[3:4, :] = dsb_
            dmr[4:5, :] = dcb

        pl.run_scoped(mlp, pltpu.VMEM((D, F), bf16), pltpu.VMEM((D, F), bf16), pltpu.VMEM((F, D), bf16),
                      pltpu.SemaphoreType.DMA((2,)))

    pl.run_scoped(phase_a, pltpu.VMEM((F, S), bf16), pltpu.VMEM((D, S), bf16),
                  pltpu.VMEM((D, S), bf16), pltpu.SemaphoreType.DMA((7 + 2 * NCH,)))

    def phase_b(do3, negd, dq3, dqa, dkv, lhs, ds0, stg, sem_b):
        cp_x = pltpu.make_async_copy(x_hbm, pc.at[1, 0], sem_b.at[2])
        cp_wq2 = pltpu.make_async_copy(wq_hbm, blk(2, 0, 0), sem_b.at[0])

        def dwm_copy(j, slot):
            return pltpu.make_async_copy(blk(slot, 1, j % 4), dwmod_hbm.at[:, j * D:(j + 1) * D], msem.at[6 + j])

        def load_copy(slot, hi_):
            return pltpu.make_async_copy(spill_hbm.at[hi_], pc.at[slot], psem.at[slot])

        cf = c_ref[...].astype(f32)
        sg = jax.nn.sigmoid(cf)
        sc_col = jnp.broadcast_to(cf * sg, (128, D)).T[:, 0:1]

        def mod_bwd(j, slot):
            row = dmr[j:j + 1, :]
            blk(slot, 1, j % 4)[...] = (sc_col * row).astype(bf16)
            dwm_copy(j, slot).start()
            wm_copy(j, slot, msem.at[j]).wait()
            return lax.dot_general(row.astype(bf16), blk(slot, 0, j % 4)[...], NT, preferred_element_type=f32)

        dwo = lax.dot_general(oT3[...].reshape(D, S), aT[...], NT, preferred_element_type=f32)
        stg[...] = dwo.astype(bf16)
        cp_dwo = pltpu.make_async_copy(stg, dwo_hbm, sem_b.at[1])
        cp_dwo.start()
        for j in range(NCH):
            cols = chunk_cols(j)
            do = jnp.dot(wo_s[...], aT[:, cols], preferred_element_type=f32).reshape(H, DH, CW)
            linv = 1.0 / l_s[:, cols]
            dob = (do * linv.reshape(H, 1, CW)).astype(bf16)
            do3[:, :, cols] = dob
            negd[:, cols] = -jnp.sum(dob.astype(f32) * oT3[:, :, cols].astype(f32), axis=1)
        dkv[...] = jnp.zeros((32, S), f32)
        dsc = mod_bwd(2, XS) + mod_bwd(3, XS) + mod_bwd(4, XS) + mod_bwd(5, XS)
        dmr[6:7, :] = dsc
        for k in range(2):
            jj = NCH - 2 + k
            pltpu.make_async_copy(stg2.at[k], dw1_hbm.at[F // 2:F, chunk_cols(jj)], sem2.at[k]).wait()

        QC, NP = 256, 2
        PC = QC // NP
        NQC = S // QC
        st_units = [(qc, g) for qc in range(NQC) for g in range(NG)]

        def make_lhs(h, par):
            lhs[par] = jnp.concatenate([do3[h], _aug(negd[pl.ds(h, 1), :])], axis=0).T

        def st_piece(slot, par, u, pi):
            qc, g = st_units[u]
            r0 = qc * QC + pi * PC
            rows = slice(r0, r0 + PC)
            dp = jnp.dot(lhs[par, rows, :], vat[:, g * QB:(g + 1) * QB], preferred_element_type=f32)
            return (pc[slot, g, rows, :].astype(f32) * dp).astype(bf16)

        def head_bwd_stored(h, slot, par, h_next, slot_next):
            cur = [ds0[pi * PC:(pi + 1) * PC, :] for pi in range(NP)]
            for u in range(len(st_units)):
                if u == 16:
                    make_lhs(h_next, 1 - par)
                qc, g = st_units[u]
                qs = slice(qc * QC, (qc + 1) * QC)
                gs = slice(g * QB, (g + 1) * QB)
                dsb = jnp.concatenate(cur, axis=0)
                nxt = []
                for pi in range(NP):
                    if u + 1 < len(st_units):
                        nxt.append(st_piece(slot, par, u + 1, pi))
                    else:
                        nxt.append(st_piece(slot_next, 1 - par, 0, pi))
                    if pi == 0:
                        dkv[16:32, gs] += jnp.dot(do3[h, :, qs], pc[slot, g, qs, :], preferred_element_type=f32)
                    else:
                        t = lax.dot_general(kT[0:16, gs], dsb, NT, preferred_element_type=f32)
                        if g == 0:
                            dqa[:, qs] = t
                        else:
                            dqa[:, qs] += t
                        dkv[0:16, gs] += jnp.dot(q3[h, :, qs], dsb, preferred_element_type=f32)
                cur = nxt
            for pi in range(NP):
                ds0[pi * PC:(pi + 1) * PC, :] = cur[pi]
            dq3[h] = (dqa[...] * 0.25).astype(bf16)

        def head_bwd_rec(h):
            CK, NP = 128, 2
            NC = S // CK
            PC = CK // NP
            units = [(g, c) for g in range(NG) for c in range(NC)]
            ws = {}

            def piece(u, pi):
                g, c = units[u]
                gc = slice(g * QB, (g + 1) * QB)
                if g not in ws:
                    z = jnp.zeros((16, QB), bf16)
                    ws[g] = jnp.concatenate([
                        jnp.concatenate([q3[h, :, gc], z], axis=1),
                        jnp.concatenate([_aug(negm[pl.ds(h, 1), gc]), _aug(negd[pl.ds(h, 1), gc])], axis=1),
                        jnp.concatenate([z, do3[h, :, gc]], axis=1)], axis=0)
                r0 = c * CK + pi * PC
                o = jnp.dot(kva[r0:r0 + PC, :], ws[g], preferred_element_type=f32)
                p = jnp.exp2(o[:, :QB])
                ds = p * o[:, QB:]
                return p.astype(bf16), ds.astype(bf16)

            cur = [piece(0, pi) for pi in range(NP)]
            dq = None
            for u in range(len(units)):
                g, c = units[u]
                gc = slice(g * QB, (g + 1) * QB)
                ks = slice(c * CK, (c + 1) * CK)
                dsb = jnp.concatenate([t[1] for t in cur], axis=0)
                pb = jnp.concatenate([t[0] for t in cur], axis=0)
                nxt = []
                for pi in range(NP):
                    if u + 1 < len(units):
                        nxt.append(piece(u + 1, pi))
                    if pi == 0:
                        dkv[16:32, ks] += lax.dot_general(do3[h, :, gc], pb, NT, preferred_element_type=f32)
                    else:
                        t = jnp.dot(kT[0:16, ks], dsb, preferred_element_type=f32)
                        dq = t if c == 0 else dq + t
                        dkv[0:16, ks] += lax.dot_general(q3[h, :, gc], dsb, NT, preferred_element_type=f32)
                if c == NC - 1:
                    dq3[h, :, gc] = (dq * 0.25).astype(bf16)
                cur = nxt

        def bwd_stored_step(i, _):
            h = tbl[4, i]
            slot = tbl[5, i]
            i_next = jnp.minimum(i + 1, N_ST - 1)
            slot_next = tbl[5, i_next]

            @pl.when(jnp.logical_and(i + 1 >= NS, i + 1 < N_ST))
            def _():
                load_copy(slot_next, 0).wait()

            head_bwd_stored(h, slot, i % 2, tbl[4, i_next], slot_next)

            @pl.when(i < N_H)
            def _():
                load_copy(slot, i).start()

            @pl.when(i == 0)
            def _():
                for j in range(2, 6):
                    dwm_copy(j, XS).wait()
                load_copy(XS, N_H).start()

            return 0

        make_lhs(tbl[4, 0], 0)
        for pi in range(NP):
            ds0[pi * PC:(pi + 1) * PC, :] = st_piece(tbl[5, 0], 0, 0, pi)
        lax.fori_loop(0, N_ST, bwd_stored_step, 0)

        cp_x.start()
        cp_wq2.start()
        for j in range(2):
            wm_copy(j, 0, msem.at[j]).start()

        if N_R > 0:
            def bwd_rec_step(i, _):
                head_bwd_rec(tbl[6, i])
                return 0

            lax.fori_loop(0, N_R, bwd_rec_step, 0)

        def stage8(xT, dkvb, xstg, sem8):
            cp_x.wait()
            cp_wq2.wait()
            cp_dwo.wait()
            wkv = jnp.concatenate([wk_ref[...], wv_ref[...], jnp.zeros((96, D), bf16)], axis=0).T
            dkvb[0:16, :] = (dkv[0:16, :] * LN2).astype(bf16)
            dkvb[16:32, :] = dkv[16:32, :].astype(bf16)
            dkvb[32:128, :] = jnp.zeros((96, S), bf16)

            def dx_copy(j):
                return pltpu.make_async_copy(xstg.at[j % 2], dx_hbm.at[pl.ds(j * CW, CW), :], sem8.at[1 + j % 2])

            dsa = dca = dw = dwkvT = None
            ca1 = jnp.broadcast_to(1.0 + col(1), (D, 128))
            for j in range(NCH):
                cols = chunk_cols(j)
                dqc = dq3[:, :, cols].reshape(D, CW)
                xT[:, cols] = pc[1, 0, cols, :].T
                dh1 = (jnp.dot(blk(2, 0, 0)[...], dqc, preferred_element_type=f32)
                       + jnp.dot(wkv, dkvb[:, cols], preferred_element_type=f32))
                blk(3, 0, j)[...] = ((xT[:, cols].astype(f32) - st[0:1, cols]) * st[1:2, cols] * (1.0 + col(1))
                                     + col(0)).astype(bf16)
                dxs = []
                for bi in range(CW // 128):
                    bc = slice(j * CW + bi * 128, j * CW + (bi + 1) * 128)
                    g = dh1[:, bi * 128:(bi + 1) * 128]
                    mean1, rstd1 = st[0:1, bc], st[1:2, bc]
                    xh = (xT[:, bc].astype(f32) - mean1) * rstd1
                    gx = g * xh
                    m1 = _colsum(g * ca1) * (1.0 / D)
                    m2 = _colsum(gx * ca1) * (1.0 / D)
                    dsa = _acc(dsa, _rowsum_blk(g))
                    dca = _acc(dca, _rowsum_blk(gx))
                    xh = (xT[:, bc].astype(f32) - mean1) * rstd1
                    dxs.append((x1T[:, bc] + rstd1 * (g * ca1 - m1 - xh * m2)).astype(bf16).T)
                dx = jnp.concatenate(dxs, axis=0)
                if j >= 2:
                    dx_copy(j - 2).wait()
                xstg[j % 2] = dx
                dx_copy(j).start()
            dmr[0:1, :] = dsa
            dmr[1:2, :] = dca
            dsc2 = dmr[6:7, :] + mod_bwd(0, 0) + mod_bwd(1, 0)
            dc_ref[...] = (dsc2 * (sg * (1.0 + cf * (1.0 - sg)))).astype(bf16)
            for j in range(NCH):
                t = lax.dot_general(dkvb[0:32, chunk_cols(j)], blk(3, 0, j)[...], NT,
                                    preferred_element_type=f32)
                dwkvT = t if dwkvT is None else dwkvT + t
            dwk_ref[...] = dwkvT[0:16].astype(bf16)
            dwv_ref[...] = dwkvT[16:32].astype(bf16)
            cp_dwq = []
            for r in range(2):
                rows = slice(r * (D // 2), (r + 1) * (D // 2))
                dw = None
                for j in range(NCH):
                    t = lax.dot_general(blk(3, 0, j)[rows, :], dq3[:, :, chunk_cols(j)].reshape(D, CW), NT,
                                        preferred_element_type=f32)
                    dw = t if dw is None else dw + t
                stg[rows, :] = dw.astype(bf16)
                cp = pltpu.make_async_copy(stg.at[rows, :], dwq_hbm.at[rows, :], sem8.at[(0, 3)[r]])
                cp.start()
                cp_dwq.append(cp)
            for j in range(NCH - 2, NCH):
                dx_copy(j).wait()
            for j in range(2):
                dwm_copy(j, 0).wait()
            for cp in cp_dwq:
                cp.wait()

        pl.run_scoped(stage8, pltpu.VMEM((D, S), bf16), pltpu.VMEM((128, S), bf16),
                      pltpu.VMEM((2, CW, D), bf16), pltpu.SemaphoreType.DMA((4,)))

    pl.run_scoped(phase_b, pltpu.VMEM((H, DH, S), bf16), pltpu.VMEM((H, S), f32), pltpu.VMEM((H, DH, S), bf16),
                  pltpu.VMEM((DH, S), f32), pltpu.VMEM((32, S), f32), pltpu.VMEM((2, S, 32), bf16),
                  pltpu.VMEM((256, QB), bf16),
                  pltpu.VMEM((D, D), bf16), pltpu.SemaphoreType.DMA((3,)))


@jax.jit
def pallas_adaLN_cond__grouped_kv_mqa__mixer_token_mlp__prompt_kernel(
    A_x: jax.Array,
    A_wq: jax.Array,
    A_wk: jax.Array,
    A_wv: jax.Array,
    A_wo: jax.Array,
    B_x: jax.Array,
    B_w1: jax.Array,
    B_b1: jax.Array,
    B_w2: jax.Array,
    B_b2: jax.Array,
    c: jax.Array,
    w_mod: jax.Array,
    grad_out: jax.Array,
):
    any_spec = pl.BlockSpec(memory_space=pl.ANY)
    vmem_spec = pl.BlockSpec(memory_space=pltpu.VMEM)
    sds = jax.ShapeDtypeStruct
    out_shape = (
        sds((S, D), bf16), sds((S, D), bf16), sds((D, D), bf16), sds((DH, D), bf16), sds((DH, D), bf16),
        sds((D, D), bf16), sds((F, S), bf16), sds((F,), bf16), sds((F, S), bf16), sds((S,), bf16),
        sds((1, D), bf16), sds((D, 6 * D), bf16), sds((N_H + 1, NG, S, QB), bf16),
    )
    out_specs = (any_spec, any_spec, any_spec, vmem_spec, vmem_spec, any_spec, any_spec, vmem_spec, any_spec,
                 vmem_spec, vmem_spec, any_spec, any_spec)
    in_specs = [any_spec, any_spec, vmem_spec, vmem_spec, any_spec, any_spec, vmem_spec, any_spec, vmem_spec,
                vmem_spec, any_spec, any_spec]
    scratch = [
        pltpu.VMEM((NS + 1, NG, S, QB), bf16),
        pltpu.VMEM((H, DH, S), bf16),
        pltpu.VMEM((H, S), f32),
        pltpu.VMEM((H, DH, S), bf16),
        pltpu.VMEM((D, S), bf16),
        pltpu.VMEM((D, S), f32),
        pltpu.VMEM((S, 48), bf16),
        pltpu.VMEM((32, S), bf16),
        pltpu.VMEM((32, S), bf16),
        pltpu.VMEM((H, S), f32),
        pltpu.VMEM((8, S), f32),
        pltpu.VMEM((D, 8), f32),
        pltpu.VMEM((8, D), f32),
        pltpu.VMEM((D, D), bf16),
        pltpu.SMEM((8, H), jnp.int32),
        pltpu.SMEM((1,), jnp.int32),
        pltpu.SemaphoreType.DMA((NS + 1,)),
        pltpu.SemaphoreType.DMA((12,)),
        pltpu.VMEM((2, F // 2, CW), bf16),
        pltpu.SemaphoreType.DMA((2,)),
    ]
    outs = pl.pallas_call(
        _kernel,
        out_shape=out_shape,
        in_specs=in_specs,
        out_specs=out_specs,
        scratch_shapes=scratch,
        compiler_params=pltpu.CompilerParams(vmem_limit_bytes=128 * 2 ** 20),
    )(A_x.reshape(S, D), A_wq, A_wk.T, A_wv.T, A_wo, B_w1.T, B_b1, B_w2, B_b2, c, w_mod,
      grad_out.reshape(S, D))
    (out, dx, dwq, dwk, dwv, dwo, dw1, db1, dw2, db2, dc, dwmod, _) = outs
    return (out.reshape(1, S, D), dx.reshape(1, S, D), dwq, dwk.T, dwv.T, dwo, dw1.T, db1, dw2, db2, dc, dwmod)
```
